```python
import os as _os
_os.environ.setdefault("JAX_PLATFORMS", "cpu")
import jax
import jax.numpy as jnp

def _softmax(x, axis=-1):
    return jax.nn.softmax(x, axis=axis)
def _gelu(x):
    return jax.nn.gelu(x, approximate=True)
def _silu(x):
    return jax.nn.silu(x)
def _sigmoid(x):
    return jax.nn.sigmoid(x)
def _layernorm(x, axis=-1, eps=1e-5):
    m = jnp.mean(x, axis=axis, keepdims=True)
    v = jnp.var(x, axis=axis, keepdims=True)
    return (x - m) / jnp.sqrt(v + eps)
def _scatter_add(tgt, idx, src, axis=0):
    return tgt.at[idx].add(src)
def _segment_sum(src, seg, n):
    return jax.ops.segment_sum(src, seg, n)
class _Rng:
    def __init__(self, key):
        self._k = key
    def _next(self):
        self._k, sub = jax.random.split(self._k)
        return sub
    def normal(self, shape):
        return jax.random.normal(self._next(), shape, dtype=jnp.bfloat16)
    def randint(self, lo, hi, shape):
        return jax.random.randint(self._next(), shape, lo, hi, dtype=jnp.int32)
    def uniform(self, shape, lo=0.0, hi=1.0):
        return jax.random.uniform(self._next(), shape, jnp.bfloat16, lo, hi)
    def permutation(self, n):
        return jax.random.permutation(self._next(), n)


kernel_name = 'standalone__geglu_ffn__prompt'

def setup_inputs():
    _rng = _Rng(jax.random.key(int.from_bytes(__import__("os").urandom(4), "little")))
    _w = (lambda a: (lambda t: t.astype(jnp.bfloat16) if jnp.issubdtype(t.dtype, jnp.floating) else t)(jnp.asarray(a)))
    B, S, D, F = 1, 2048, 576, 4608
    return {
        "x": _w((lambda *s: _rng.normal(s) * 0.05)(B, S, D)),
        "w_gate": _w((lambda *s: _rng.normal(s) * 0.05)(D, F)),
        "w_up": _w((lambda *s: _rng.normal(s) * 0.05)(D, F)),
        "w_down": _w((lambda *s: _rng.normal(s) * 0.05)(F, D)),
    }

def reference(x, w_gate, w_up, w_down):
    return (_gelu(x @ w_gate) * (x @ w_up)) @ w_down
```

```python
import functools

import jax
import jax.numpy as jnp
import numpy as np
from jax import lax
from jax.experimental import pallas as pl
from jax.experimental.pallas import tpu as pltpu

F32, BF16, U32 = jnp.float32, jnp.bfloat16, jnp.uint32
NT = (((1,), (1,)), ((), ()))
C1 = float(np.sqrt(2 / np.pi))
C2 = C1 * 0.044715
L = 128
TS, TF = 512, 512
NQ, NC = TF // L, TS // L


def _act2(g, u):
    t = jnp.tanh(g * (C1 + C2 * (g * g)))
    gu = g * u
    return gu * t + gu


def _anchor(tiles, items, never):
    nk, nr = len(tiles), tiles[0].shape[0] // 8
    pos = {}
    for n, (slot, v) in enumerate(items):
        pos.setdefault((n % nk, slot), []).append(v)
    out = []
    for k, tile in enumerate(tiles):
        pieces, done = [], 0
        for slot in range(nr):
            if (k, slot) in pos:
                if slot > done:
                    pieces.append(tile[done * 8:slot * 8])
                v = tile[slot * 8:slot * 8 + 8]
                for it in pos[k, slot]:
                    v = jnp.where(never, it if it.dtype == U32 else pltpu.bitcast(it, U32), v)
                pieces.append(v)
                done = slot + 1
        if done < nr:
            pieces.append(tile[done * 8:])
        out.append(pltpu.bitcast(jnp.concatenate(pieces, axis=0) if len(pieces) > 1 else pieces[0], BF16))
    return jnp.concatenate(out, axis=1) if nk > 1 else out[0]


def _plan(d, kt, rs, extras, tail_first=True, act_w=12, tail_w=10, lead=6, margin=10, cmargin=40,
          nseg=4, last_end=NC - 1):
    ns = len(rs)
    dots = []
    for i in range(ns):
        for g in range(2):
            tail = [("t", i, g, (TS - rs[i]) // 16)]
            main = [("gu"[g], i, q, TS // 16) for q in range(NQ)]
            dots += tail + main if (tail_first or i or g) else main + tail
        if i:
            dots += [("d", i - 1, s, d // 16) for s in range(NC)]
    dots += [("d", ns - 1, s, d // 16) for s in range(NC)]
    start = np.concatenate([[0], np.cumsum([t[3] for t in dots])])
    idx = {t[:3]: n for n, t in enumerate(dots)}
    load = np.concatenate([np.full(t[3], tail_w if t[0] == "t" else 8.0) for t in dots])
    at = {}
    for i in range(ns):
        nm = (TS - rs[i]) // 8
        t0 = start[idx["u", i, 1]]
        if i + 1 < ns:
            t1 = start[idx["u", i + 1, 1]]
            order = [(q, m) for q in range(NQ) for m in range(nm)]
        else:
            t1 = start[idx["d", i, last_end]] - margin
            order = [(q, m) for s in range(NC) for q in range(NQ) for m in range(s * 16, min(s * 16 + 16, nm))]
        order += [(q, m) for q in range(NQ) for m in range(nm, TS // 8)]
        for n, (q, m) in enumerate(order):
            after = idx["u", i, q] + 1
            t = int(t0 + (n + 0.5) / len(order) * (t1 - t0))
            t = max(t, start[after] + (m // 2) * dots[after][3] // (TS // 16))
            t = min(t, start[idx["d", i, m // 16]] - margin)
            at["h", i, q, m] = t
            load[t] += act_w
    for e, (pieces, w, first, last) in enumerate(extras):
        t0, t1 = start[idx[first]], start[idx[last] + 1]
        for n in range(len(pieces)):
            t = min(int(t0 + (n + 1) / len(pieces) * (t1 - t0)), t1 - 1)
            at["x", e, n] = t
            load[t] += w
    chains = [("ch", i, q, m, sg) for i in range(ns) for q in range(NQ)
              for m in range((TS - rs[i]) // 8, TS // 8, 2) for sg in range(nseg)]
    if chains:
        i = chains[-1][1]
        end = min(at["h", i, q, (TS - rs[i]) // 8] for q in range(NQ)) + cmargin
        level = np.convolve(load, np.ones(8) / 8, mode="same")[:end]
        level[:lead if isinstance(lead, int) else start[idx[lead]]] = 1e9
        work = 4 * (2 * kt // nseg + 1)
        lo, hi = 0.0, 1e3
        for _ in range(50):
            mid = (lo + hi) / 2
            lo, hi = (mid, hi) if np.maximum(mid - level, 0).sum() < work * len(chains) else (lo, mid)
        room = np.cumsum(np.maximum(hi - level, 0))
        for n, c in enumerate(chains):
            at[c] = min(int(np.searchsorted(room, (n + 1) * work - 1e-6)), at["h", c[1], c[2], c[3]])
    per = [[] for _ in dots]
    for item, t in sorted(at.items(), key=lambda kv: kv[1]):
        n = int(np.searchsorted(start, t, side="right")) - 1
        per[n].append((int(t - start[n]), item))
    return dots, per, nseg


def _kernel(xt_h, wg_h, wu_h, wdt_h, ot_h,
            xt_v, x_v, xb_v, w_v, wtb_v, wt_v, acc_v, o_v, zero_s,
            sem_x, sem_g0, sem_w, sem_b, sem_o, *, cfg):
    d, s_len = xt_h.shape
    k0 = d // L * L
    kt, nk = d - k0, k0 // L
    ns, nf, half = s_len // TS, wg_h.shape[1] // TF, TS // 2
    r = xb_v.shape[2]

    def copy_x(i):
        sem = sem_x.at[min(i, 2)] if i < 4 else sem_b
        return pltpu.make_async_copy(xt_h.at[:, pl.ds(i * half, half)], xt_v.at[i], sem)

    def copy_g0(q):
        return pltpu.make_async_copy(wg_h.at[:, pl.ds(q * L, L)], w_v.at[0, 0, :, pl.ds(q * L, L)], sem_g0.at[q])

    def copy_w(j, n):
        sem = sem_b if (j, n) == (0, 2) else sem_w.at[j]
        return pltpu.make_async_copy((wg_h, wu_h, wdt_h)[n].at[:, pl.ds(j * TF, TF)], w_v.at[j, n], sem)

    def copy_tail(g):
        return pltpu.make_async_copy((wg_h, wu_h)[g].at[pl.ds(k0, kt), :], wtb_v.at[g], sem_b)

    def copy_out(c, s):
        return pltpu.make_async_copy(o_v.at[c, s], ot_h.at[:, pl.ds(c * TS + s * L, L)], sem_o)

    def group(*js):
        return [copy_w(j, n) for j in js for n in range(3)]

    def dma(wait=(), start=()):
        def run():
            for cp in wait:
                cp.wait()
            for cp in start:
                cp.start()
        return run

    def transpose_piece(i, k, s):
        if k < nk:
            blk = xt_v[i, k * L:(k + 1) * L, s * L:(s + 1) * L]
        else:
            blk = jnp.concatenate([xt_v[i, k0:, s * L:(s + 1) * L], jnp.zeros((L - kt, L), BF16)], axis=0)
        v = pltpu.bitcast(blk.T, U32)
        row = (i % 2 * half + s * L) // 2
        x_v[i // 2, k, row:row + L // 2] = v
        return v

    def transpose_pieces(*halves):
        return [functools.partial(transpose_piece, i, k, s)
                for i in halves for s in range(half // L) for k in range(nk + 1)]

    def splat_pieces(c, per=4):
        cols = []

        def piece(n):
            if not cols:
                cols.append(xt_v[2 * c + 1, k0:, half - L:].astype(F32).T[L - r:])
            for k in range(n * per, (n + 1) * per):
                v = jnp.broadcast_to(cols[0][:, k:k + 1], (r, L))
                xb_v[c, k] = v
            return v
        return [functools.partial(piece, n) for n in range(kt // per)]

    def tail_piece(g, j):
        v = wtb_v[g, :, j * TF:(j + 1) * TF].astype(F32)
        wt_v[g, j] = v
        return v

    def zero_piece(c, s):
        acc_v[c, s] = jnp.zeros((d, L), F32)

    def out_piece(c, s):
        v = 0.5 * acc_v[c, s]
        o_v[c, s] = v.astype(BF16)
        return v

    masks = [0]

    def all_false():
        masks[0] += 1
        return jnp.broadcast_to(lax.rem(zero_s[0] + masks[0], nf), (8, L)) < 0

    def run_steps(steps, rs, extras=(), before=None, after=None, init=False, final=False, **plan_args):
        before, after = before or {}, after or {}
        dots, per, nseg = _plan(d, kt, rs, extras, **plan_args)
        res, val = {}, {}

        def vpu_tail(i, q, m, sg):
            c, j = steps[i]
            row = m * 8 - (TS - r)
            acc = val["ch", i, q, m, sg - 1] if sg else [None, None]
            for k in range(sg * kt // nseg, (sg + 1) * kt // nseg):
                xb = xb_v[c, k, row:row + 16, :]
                p = [xb * wt_v[g, j, k:k + 1, q * L:(q + 1) * L] for g in range(2)]
                acc = [p[g] if acc[g] is None else acc[g] + p[g] for g in range(2)]
            return acc

        def activation(i, q, m, token, never):
            main = [res["gu"[g], i, q][m * 8:m * 8 + 8] for g in range(2)]
            if m >= (TS - rs[i]) // 8:
                tail = val["ch", i, q, m // 2 * 2, nseg - 1]
                return _act2(*[jnp.where(never, token, main[g]) + tail[g][m % 2 * 8:m % 2 * 8 + 8] for g in range(2)])
            tail = [res["t", i, g][m * 8:m * 8 + 8, q * L:(q + 1) * L] for g in range(2)]
            return _act2(jnp.where(never, token, main[0] + tail[0]), main[1] + tail[1])

        prev = wd = never = None
        for (kind, i, n, slots), items in zip(dots, per):
            c, j = steps[i]
            if (kind, i, n) in before:
                before[kind, i, n]()
            if (kind, i, n) in before or prev is None:
                never = all_false()
            tied = []
            for slot, item in items:
                if item[0] == "ch":
                    v = val[item] = vpu_tail(*item[1:])
                    tied += [(slot, v[g][h:h + 8]) for h in (0, 8) for g in range(2)]
                elif item[0] == "x":
                    v = extras[item[1]][0][item[2]]()
                    if v is not None:
                        tied.append((slot, v[-8:, -L:]))
                else:
                    row = slot * prev.shape[0] // (slots * 8) * 8
                    v = val[item] = activation(*item[1:], prev[row:row + 8, -L:], never)
                    tied.append((slot, v))
            if kind == "t":
                lhs = _anchor([x_v[c, nk, :(TS - rs[i]) // 2]], tied, never)[:, :kt]
                out = jnp.dot(lhs, w_v[j, n, k0:, :], preferred_element_type=F32)
            elif kind == "d":
                if n == 0:
                    wd = [pltpu.bitcast(w_v[j, 2, :, q * L:(q + 1) * L], U32) for q in range(NQ)]
                h = jnp.concatenate(
                    [jnp.concatenate([val["h", i, q, n * 16 + m] for m in range(16)], axis=0) for q in range(NQ)],
                    axis=1)
                out = lax.dot_general(_anchor(wd, tied, never), h.astype(BF16), NT, preferred_element_type=F32)
                if not init:
                    out = acc_v[c, n] + out
                if final:
                    o_v[c, n] = (0.5 * out).astype(BF16)
                else:
                    acc_v[c, n] = out
            else:
                lhs = _anchor([x_v[c, k] for k in range(nk)], tied, never)
                out = jnp.dot(lhs, w_v[j, "gu".index(kind), :k0, n * L:(n + 1) * L], preferred_element_type=F32)
            if (kind, i, n) in after:
                after[kind, i, n]()
            res[kind, i, n] = prev = out

    def once(fn):
        lax.fori_loop(0, zero_s[0] + 1, lambda t, carry: fn(), None)

    copy_x(0).start()
    copy_x(1).start()
    zero_s[0] = 0
    for i in range(2):
        dma([copy_x(i)], [copy_g0(2 * i), copy_g0(2 * i + 1)])()
        for piece in transpose_pieces(i):
            piece()
    bulk = [copy_w(0, 2), copy_tail(0), copy_tail(1)] + [copy_x(i) for i in range(4, 2 * ns)]
    once(lambda: run_steps(
        [(0, 0), (1, 0)], cfg["r_first"],
        extras=[
            ([functools.partial(zero_piece, c, s) for c in (2, 3) for s in range(NC)], 0, ("g", 0, 1), ("g", 0, 3)),
            (transpose_pieces(2, 3), 40, ("u", 0, 1), ("u", 0, 2)),
            (splat_pieces(0) + splat_pieces(1), 10, ("u", 0, 3), ("g", 1, 3)),
            (transpose_pieces(4, 5, 6, 7), 40, ("u", 1, 1), ("u", 1, 3)),
            (splat_pieces(2) + splat_pieces(3), 10, ("d", 0, 0), ("d", 1, 1)),
            ([functools.partial(tail_piece, g, j) for j in range(nf) for g in range(2)], 40, ("d", 1, 0), ("d", 1, 3)),
        ],
        before={
            ("g", 0, 0): dma([copy_g0(0)], [copy_w(0, 1)]),
            ("g", 0, 1): dma([copy_g0(1)], [copy_x(2), copy_x(3)]),
            ("g", 0, 2): dma([copy_g0(2), copy_g0(3)], bulk),
            ("t", 0, 1): dma([copy_w(0, 1)], group(1)),
            ("u", 0, 1): dma([copy_x(2), copy_x(3)], group(2)),
            ("u", 1, 1): dma(bulk, group(*range(3, nf))),
        },
        init=True, tail_first=False, **cfg["first"]))

    def body(t, carry):
        for tt in range(nf // 2):
            pl.when(t == tt)(dma(group(1 + 2 * tt, 2 + 2 * tt)))
        steps = []
        for e in (1, 2):
            p = (2 * t + e >= nf).astype(jnp.int32)
            steps += [(2 * p + c, 2 * t + e - nf * p) for c in range(2)]
        run_steps(steps, cfg["r_loop"], **cfg["loop"])

    lax.fori_loop(0, nf - 1, body, None)

    after = {("g", 0, 3): dma(start=[copy_out(c, s) for c in range(2) for s in range(NC)])}
    after.update({("d", i, s): dma(start=[copy_out(2 + i, s)]) for i in range(2) for s in range(NC)})
    once(lambda: run_steps(
        [(2, nf - 1), (3, nf - 1)], cfg["r_last"],
        extras=[([functools.partial(out_piece, c, s) for c in range(2) for s in range(NC)], 120,
                 ("t", 0, 0), ("g", 0, 3))],
        after=after, final=True, **cfg["last"]))
    dma([copy_out(c, s) for c in range(ns) for s in range(NC)])()


CONFIG = dict(r_first=(0, 0), r_loop=(96, 96, 96, 96), r_last=(64, 64), first={}, loop={}, last={})


def _geglu(x, w_gate, w_up, w_down, cfg):
    b, s, d = x.shape
    f = w_gate.shape[1]
    assert b * s == 4 * TS and f % TF == 0 and (f // TF) % 2 == 1 and d % L == L // 2
    ns, nf, kt = b * s // TS, f // TF, d % L
    r = max(cfg["r_first"] + cfg["r_loop"] + cfg["r_last"] + (16,))
    vmem, sem = pltpu.VMEM, pltpu.SemaphoreType.DMA
    out_t = pl.pallas_call(
        functools.partial(_kernel, cfg=cfg),
        in_specs=[pl.BlockSpec(memory_space=pl.ANY)] * 4,
        out_specs=pl.BlockSpec(memory_space=pl.ANY),
        out_shape=jax.ShapeDtypeStruct((d, b * s), x.dtype),
        scratch_shapes=[
            vmem((2 * ns, d, TS // 2), BF16),
            vmem((ns, d // L + 1, TS // 2, L), U32),
            vmem((ns, kt, r, L), F32),
            vmem((nf, 3, d, TF), BF16),
            vmem((2, kt, f), BF16),
            vmem((2, nf, kt, TF), F32),
            vmem((ns, NC, d, L), F32),
            vmem((ns, NC, d, L), BF16),
            pltpu.SMEM((1,), jnp.int32),
            sem((3,)), sem((NQ,)), sem((nf,)), sem(()), sem(()),
        ],
        compiler_params=pltpu.CompilerParams(vmem_limit_bytes=100 * 1024 * 1024),
    )(x.reshape(b * s, d).T, w_gate, w_up, w_down.T)
    return out_t.T.reshape(b, s, d)


@jax.jit
def pallas_standalone__geglu_ffn__prompt_kernel(
    x: jax.Array,
    w_gate: jax.Array,
    w_up: jax.Array,
    w_down: jax.Array,
):
    return _geglu(x, w_gate, w_up, w_down, CONFIG)
```

```python
import functools

import jax
import jax.numpy as jnp
import numpy as np
from jax import lax
from jax.experimental import pallas as pl
from jax.experimental.pallas import tpu as pltpu

F32, BF16, U32 = jnp.float32, jnp.bfloat16, jnp.uint32
NT = (((1,), (1,)), ((), ()))
C1 = float(np.sqrt(2 / np.pi))
C2 = C1 * 0.044715
L = 128
TS, TF = 512, 512
NQ, NC = TF // L, TS // L
R, R_LAST = 96, 80
NSEG = 4
CUT = 448


def _act2(g, u):
    t = jnp.tanh(g * (C1 + C2 * (g * g)))
    gu = g * u
    return gu * t + gu


def _tie(never, other, v):
    return jnp.where(never, other if other.dtype == v.dtype else pltpu.bitcast(other, v.dtype), v)


def _tie_rows(tie, v):
    return jnp.concatenate([tie(v[n:n + 8]) for n in range(0, v.shape[0], 8)], axis=0)


def _lhs(tiles, tied, never):
    waits = {}
    for n, (slot, v) in enumerate(tied):
        waits.setdefault((n % len(tiles), slot), []).append(v)
    cols = []
    for k, tile in enumerate(tiles):
        pieces, done = [], 0
        for slot in range(tile.shape[0] // 8):
            if (k, slot) in waits:
                if slot > done:
                    pieces.append(tile[done * 8:slot * 8])
                v = tile[slot * 8:slot * 8 + 8]
                for other in waits[k, slot]:
                    v = _tie(never, other, v)
                pieces.append(v)
                done = slot + 1
        if done * 8 < tile.shape[0]:
            pieces.append(tile[done * 8:])
        cols.append(pltpu.bitcast(jnp.concatenate(pieces, axis=0), BF16))
    return jnp.concatenate(cols, axis=1)


def _plan(d, kt, steps, r, extras, quiet, startup, lead):
    margin, nm = 10, (TS - r) // 8
    dots = []
    for i in range(steps):
        for g in range(2):
            tail = [("t", i, g, (TS - r) // 16)]
            main = [("gu"[g], i, q, TS // 16) for q in range(NQ)]
            dots += main + tail if startup and (i, g) == (0, 0) else tail + main
        if i:
            dots += [("d", i - 1, s, d // 16) for s in range(NC)]
    dots += [("d", steps - 1, s, d // 16) for s in range(NC)]
    start = np.concatenate([[0], np.cumsum([t[3] for t in dots])])
    idx = {t[:3]: n for n, t in enumerate(dots)}
    load = np.concatenate([np.full(t[3], 10.0 if t[0] == "t" else 8.0) for t in dots])
    usable = np.concatenate([np.full(t[3], t[:3] not in quiet) for t in dots])

    def spread(t0, t1, frac):
        free = t0 + np.flatnonzero(usable[t0:t1])
        return int(free[min(int(frac * len(free)), len(free) - 1)])

    at = {}
    for i in range(steps):
        t0 = start[idx["u", i, 1]]
        if i + 1 < steps and not startup:
            t1 = start[idx["u", i + 1, 1]]
            order = [(q, m) for q in range(NQ) for m in range(nm)]
        else:
            t1 = start[idx["d", i, NC - 1]] - margin
            order = [(q, m) for s in range(NC) for q in range(NQ) for m in range(s * 16, min(s * 16 + 16, nm))]
        order += [(q, m) for q in range(NQ) for m in range(nm, TS // 8)]
        for n, (q, m) in enumerate(order):
            after = idx["u", i, q] + 1
            t = spread(t0, t1, (n + 0.5) / len(order))
            t = max(t, start[after] + (m // 2) * dots[after][3] // (TS // 16))
            t = min(t, start[idx["d", i, m // 16]] - margin)
            at["h", i, q, m] = t
            load[t] += 12
    for e, (pieces, weight, first, last) in enumerate(extras):
        for n in range(len(pieces)):
            t = spread(start[idx[first]], start[idx[last] + 1], (n + 1) / len(pieces))
            at["x", e, n] = t
            load[t] += weight
    tails = [("ch", i, q, m, sg) for i in range(steps) for q in range(NQ)
             for m in range(nm, TS // 8, 2) for sg in range(NSEG)]
    if tails:
        end = min(at["h", steps - 1, q, nm] for q in range(NQ)) + 40
        level = np.convolve(load, np.ones(8) / 8, mode="same")[:end]
        level[:lead] = 1e9
        work = 4 * (2 * kt // NSEG + 1)
        lo, hi = 0.0, 1e3
        for _ in range(50):
            mid = (lo + hi) / 2
            lo, hi = (mid, hi) if np.maximum(mid - level, 0).sum() < work * len(tails) else (lo, mid)
        room = np.cumsum(np.maximum(hi - level, 0))
        for n, c in enumerate(tails):
            at[c] = min(int(np.searchsorted(room, (n + 1) * work - 1e-6)), at["h", c[1], c[2], c[3]] - 1)
    items = [[] for _ in dots]
    for item, t in sorted(at.items(), key=lambda kv: kv[1]):
        n = int(np.searchsorted(start, t, side="right")) - 1
        items[n].append((int(t - start[n]), item))
    return dots, items


def _kernel(xt_h, wg_h, wu_h, wdt_h, ot_h,
            xt_v, x_v, xs_v, w_v, wtb_v, wt_v, acc_v, o_v, zero_s,
            sem_q, sem_g, sem_x, sem_w, sem_b, sem_o):
    d, s_len = xt_h.shape
    k0 = d // L * L
    kt, nk = d - k0, k0 // L
    ns, nf, half = s_len // TS, wg_h.shape[1] // TF, TS // 2
    copy = pltpu.make_async_copy

    def copy_x(i):
        return copy(xt_h.at[:, pl.ds(i * half, half)], xt_v.at[i], sem_x if i < 4 else sem_b)

    def copy_g0(q):
        return copy(wg_h.at[pl.ds(0, k0), pl.ds(q * L, L)], w_v.at[0, 0, pl.ds(0, k0), pl.ds(q * L, L)],
                    sem_g.at[min(q, 2)])

    def copy_w(j, n):
        return copy((wg_h, wu_h, wdt_h)[n].at[:, pl.ds(j * TF, TF)], w_v.at[j, n],
                    sem_b if (j, n) == (0, 2) else sem_w.at[(j + 1) // 2])

    def copy_tail(g):
        return copy((wg_h, wu_h)[g].at[pl.ds(k0, kt), pl.ds(TF, (nf - 1) * TF)], wtb_v.at[g], sem_b)

    def out_parts(c, s):
        return [(0, CUT), (CUT, d - CUT)] if (c, s) == (ns - 1, NC - 1) else [(0, d)]

    def copy_out(c, s, row, rows):
        return copy(o_v.at[c * NC + s, pl.ds(row, rows)],
                    ot_h.at[pl.ds(row, rows), pl.ds(c * TS + s * L, L)], sem_o)

    def group(j):
        return [copy_w(j, n) for n in range(3)]

    def dma(wait=(), start=()):
        def run():
            for cp in wait:
                cp.wait()
            for cp in start:
                cp.start()
        return run

    def transpose_piece(i, s, k, tie=None):
        if k < nk:
            blk = xt_v[i, k * L:(k + 1) * L, s * L:(s + 1) * L]
        else:
            blk = jnp.concatenate([xt_v[i, k0:, s * L:(s + 1) * L], jnp.zeros((L - kt, L), BF16)], axis=0)
        if tie is not None:
            blk = pltpu.bitcast(_tie_rows(tie, pltpu.bitcast(blk, U32)), BF16)
        v = pltpu.bitcast(blk.T, U32)
        row = (i % 2 * half + s * L) // 2
        x_v[i // 2, k, row:row + L // 2] = v
        return v

    def transpose_pieces(*halves):
        return [functools.partial(transpose_piece, i, s, k)
                for i in halves for s in range(half // L) for k in range(nk + 1)]

    def splat_piece(c, first, tie):
        src = _tie_rows(tie, x_v[c, nk, (TS - R) // 2:TS // 2])
        for k in range(first, first + 4):
            v = pltpu.bitcast(jnp.broadcast_to(src[:, k:k + 1], (R // 2, L)), BF16).astype(F32)
            xs_v[c, k, :R] = v
        return v

    def splat_pieces(c):
        return [functools.partial(splat_piece, c, k) for k in range(0, kt, 4)]

    def tail_cols(g, q):
        return slice((2 * q + g) * L, (2 * q + g + 1) * L)

    def tail_piece(j, g, tie):
        v = (wtb_v[g, :, (j - 1) * TF:j * TF] if j else w_v[0, g, k0:, :]).astype(F32)
        for q in range(NQ):
            col = _tie_rows(tie, v[:, q * L:(q + 1) * L])
            wt_v[j, :, tail_cols(g, q)] = col
        return col

    def zero_piece(c, s, part, tie):
        rows = d // 4
        acc_v[c, s, part * rows:(part + 1) * rows] = jnp.concatenate(
            [tie(jnp.zeros((8, L), F32))] * (rows // 8), axis=0)

    def out_piece(c, s, tie):
        del tie
        o_v[c * NC + s] = (0.5 * acc_v[c, s]).astype(BF16)
        return pltpu.bitcast(o_v[c * NC + s + zero_s[0], :16], U32)

    masks = []

    def all_false():
        masks.append(None)
        return jnp.broadcast_to(lax.rem(zero_s[0] + len(masks), nf), (8, L)) < 0

    def run_steps(steps, r, extras=(), before=None, after=None, quiet=(), startup=False, final=False, lead=6):
        before, after = before or {}, after or {}
        dots, items = _plan(d, kt, len(steps), r, extras, quiet, startup, lead)
        res, val = {}, {}

        def weight(j, n, rows):
            return [pltpu.bitcast(w_v[j, n, rows, q * L:(q + 1) * L], U32) for q in range(NQ)]

        def vpu_tail(i, q, m, sg):
            c, j = steps[i]
            row = m * 8 - (TS - R)
            acc = val["ch", i, q, m, sg - 1] if sg else None
            for k in range(sg * kt // NSEG, (sg + 1) * kt // NSEG):
                xs = xs_v[c, k, row:row + 16, :]
                p = [xs * wt_v[j, k:k + 1, tail_cols(g, q)] for g in range(2)]
                acc = p if acc is None else [a + b for a, b in zip(acc, p)]
            return acc

        def activation(i, q, m, tie):
            main = [res["gu"[g], i, q][m * 8:m * 8 + 8] for g in range(2)]
            if m >= (TS - r) // 8:
                tail = val["ch", i, q, m // 2 * 2, NSEG - 1]
                return _act2(*[tie(main[g]) + tail[g][m % 2 * 8:m % 2 * 8 + 8] for g in range(2)])
            tail = [res["t", i, g][m * 8:m * 8 + 8, q * L:(q + 1) * L] for g in range(2)]
            return _act2(tie(main[0] + tail[0]), main[1] + tail[1])

        prev = wd = never = tie = None
        for (kind, i, n, slots), todo in zip(dots, items):
            c, j = steps[i]
            if (kind, i, n) in before:
                before[kind, i, n]()
            if (kind, i, n) in before or prev is None:
                never = all_false()
            tied = []
            for slot, item in todo:
                if prev is not None:
                    row = slot * prev.shape[0] // (slots * 8) * 8
                    tie = functools.partial(_tie, never, prev[row:row + 8, -L:])
                if item[0] == "ch":
                    v = val[item] = vpu_tail(*item[1:])
                    tied += [(slot, v[g][h:h + 8]) for h in (0, 8) for g in range(2)]
                elif item[0] == "h":
                    v = val[item] = activation(*item[1:], tie)
                    tied.append((slot, v))
                else:
                    v = extras[item[1]][0][item[2]](tie)
                    if v is not None:
                        tied.append((slot, v[-8:]))
            if kind == "t":
                lhs = _lhs([x_v[c, nk, :(TS - r) // 2]], tied, never)[:, :kt]
                out = jnp.dot(lhs, w_v[j, n, k0:, :], preferred_element_type=F32)
            elif kind == "d":
                if n == 0:
                    wd = weight(j, 2, slice(0, d))
                h = jnp.concatenate(
                    [jnp.concatenate([val["h", i, q, n * 16 + m] for m in range(16)], axis=0) for q in range(NQ)],
                    axis=1)
                out = lax.dot_general(_lhs(wd, tied, never), h.astype(BF16), NT, preferred_element_type=F32)
                if not startup:
                    out = acc_v[c, n] + out
                if final:
                    for row, rows in out_parts(c, n):
                        o_v[c * NC + n, row:row + rows] = (0.5 * out[row:row + rows]).astype(BF16)
                        copy_out(c, n, row, rows).start()
                else:
                    acc_v[c, n] = out
            else:
                lhs = _lhs([x_v[c, k, :TS // 2] for k in range(nk)], tied, never)
                out = jnp.dot(lhs, w_v[j, "gu".index(kind), :k0, n * L:(n + 1) * L], preferred_element_type=F32)
            if (kind, i, n) in after:
                after[kind, i, n]()
            res[kind, i, n] = prev = out

    def once(fn):
        lax.fori_loop(0, zero_s[0] + 1, lambda t, carry: fn(), None)

    zero_s[0] = 0
    head = [copy(xt_h.at[pl.ds(0, k0), pl.ds(n * L, L)],
                 xt_v.at[n // 2, pl.ds(0, k0), pl.ds(n % 2 * L, L)], sem_q.at[n]) for n in range(NC)]
    rest = [copy_g0(2), copy_g0(3),
            copy(wg_h.at[pl.ds(k0, kt), pl.ds(0, TF)], w_v.at[0, 0, pl.ds(k0, kt)], sem_g.at[2])]
    rest += [copy(xt_h.at[pl.ds(k0, kt), pl.ds(i * half, half)], xt_v.at[i, pl.ds(k0, kt)], sem_g.at[2])
             for i in range(2)]
    dma(start=head[:3])()
    for n, then in enumerate([[head[3]], [copy_g0(0)], [copy_g0(1)], rest]):
        dma([head[n]], then)()
        for k in range(nk):
            transpose_piece(n // 2, n % 2, k)

    bulk = [copy_w(0, 2), copy_tail(0), copy_tail(1)] + [copy_x(i) for i in range(4, 2 * ns)]
    once(lambda: run_steps(
        [(0, 0), (1, 0)], 0,
        extras=[
            ([functools.partial(transpose_piece, n // 2, n % 2, nk) for n in range(NC)], 40,
             ("g", 0, 3), ("g", 0, 3)),
            (splat_pieces(0)[:8], 10, ("u", 0, 0), ("u", 0, 0)),
            (transpose_pieces(2, 3), 40, ("u", 0, 2), ("u", 0, 3)),
            (splat_pieces(0)[8:] + splat_pieces(1), 10, ("t", 1, 0), ("u", 1, 0)),
            ([functools.partial(zero_piece, c, s, p) for c in (2, 3) for s in range(NC) for p in range(4)], 0,
             ("g", 1, 0), ("g", 1, 3)),
            (transpose_pieces(4, 5, 6, 7), 40, ("u", 1, 2), ("d", 0, 0)),
            (splat_pieces(2) + splat_pieces(3), 10, ("d", 0, 1), ("d", 1, 3)),
            ([functools.partial(tail_piece, j, g) for j in range(nf) for g in range(2)], 40,
             ("u", 1, 2), ("d", 0, 3)),
        ],
        before={
            ("g", 0, 0): dma([copy_g0(0)], [copy_w(0, 1)]),
            ("g", 0, 1): dma([copy_g0(1)], [copy_x(2), copy_x(3)]),
            ("g", 0, 2): dma(rest, bulk[3:5]),
            ("t", 0, 1): dma([copy_w(0, 1)], bulk[:3]),
            ("u", 0, 1): dma([copy_x(2), copy_x(3)]),
            ("u", 1, 1): dma(bulk),
        },
        after={
            ("g", 0, 3): dma(start=bulk[5:]),
            ("u", 0, 3): dma(start=group(1)),
            ("g", 1, 1): dma(start=group(2)),
            **{("d", n // NC, n % NC): dma(start=group(3 + n)) for n in range(nf - 3)},
        },
        quiet=[("u", 0, 1), ("u", 1, 1)], startup=True))

    def block(n):
        p = (n >= nf).astype(jnp.int32)
        return p, n - nf * p

    def body(t, carry):
        @pl.when(t < nf // 2)
        def _():
            pair = w_v.at[pl.ds(2 * t + 1, 2)]
            copy(pair, pair, sem_w.at[t + 1]).wait()

        run_steps([(2 * p + c, j) for p, j in (carry, block(2 * t + 2)) for c in range(2)], R, lead=4)
        return block(2 * t + 3)

    lax.fori_loop(0, nf - 1, body, (jnp.int32(0), jnp.int32(1)))

    once(lambda: run_steps(
        [(2, nf - 1), (3, nf - 1)], R_LAST,
        extras=[([functools.partial(out_piece, c, s) for c in range(2) for s in range(NC)], 120,
                 ("g", 0, 0), ("u", 0, 0))],
        after={("u", 0, 0): dma(start=[copy_out(c, s, 0, d) for c in range(2) for s in range(NC)])},
        final=True))
    dma([copy_out(c, s, *part) for c in range(ns) for s in range(NC) for part in out_parts(c, s)])()


@jax.jit
def pallas_standalone__geglu_ffn__prompt_kernel(
    x: jax.Array,
    w_gate: jax.Array,
    w_up: jax.Array,
    w_down: jax.Array,
):
    b, s, d = x.shape
    f = w_gate.shape[1]
    assert (b * s, d, f) == (4 * TS, 576, 9 * TF)
    ns, nf, kt = b * s // TS, f // TF, d % L
    vmem, sem = pltpu.VMEM, pltpu.SemaphoreType.DMA
    out_t = pl.pallas_call(
        _kernel,
        in_specs=[pl.BlockSpec(memory_space=pl.ANY)] * 4,
        out_specs=pl.BlockSpec(memory_space=pl.ANY),
        out_shape=jax.ShapeDtypeStruct((d, b * s), x.dtype),
        scratch_shapes=[
            vmem((2 * ns, d, TS // 2), BF16),
            vmem((ns, d // L + 1, TS // 2 + 16, L), U32),
            vmem((ns, kt, R + 8, L), F32),
            vmem((nf, 3, d, TF), BF16),
            vmem((2, kt, f - TF), BF16),
            vmem((nf, kt, 2 * TF + L), F32),
            vmem((ns, NC, d, L), F32),
            vmem((ns * NC, d, L), BF16),
            pltpu.SMEM((1,), jnp.int32),
            sem((NC,)), sem((3,)), sem(()), sem((nf // 2 + 1,)), sem(()), sem(()),
        ],
        compiler_params=pltpu.CompilerParams(vmem_limit_bytes=100 * 1024 * 1024),
    )(x.reshape(b * s, d).T, w_gate, w_up, w_down.T)
    return out_t.T.reshape(b, s, d)
```
